```python
import os as _os
_os.environ.setdefault("JAX_PLATFORMS", "cpu")
import jax
import jax.numpy as jnp

def _softmax(x, axis=-1):
    return jax.nn.softmax(x, axis=axis)
def _gelu(x):
    return jax.nn.gelu(x, approximate=True)
def _silu(x):
    return jax.nn.silu(x)
def _sigmoid(x):
    return jax.nn.sigmoid(x)
def _layernorm(x, axis=-1, eps=1e-5):
    m = jnp.mean(x, axis=axis, keepdims=True)
    v = jnp.var(x, axis=axis, keepdims=True)
    return (x - m) / jnp.sqrt(v + eps)
def _scatter_add(tgt, idx, src, axis=0):
    return tgt.at[idx].add(src)
def _segment_sum(src, seg, n):
    return jax.ops.segment_sum(src, seg, n)
class _Rng:
    def __init__(self, key):
        self._k = key
    def _next(self):
        self._k, sub = jax.random.split(self._k)
        return sub
    def normal(self, shape):
        return jax.random.normal(self._next(), shape, dtype=jnp.bfloat16)
    def randint(self, lo, hi, shape):
        return jax.random.randint(self._next(), shape, lo, hi, dtype=jnp.int32)
    def uniform(self, shape, lo=0.0, hi=1.0):
        return jax.random.uniform(self._next(), shape, jnp.bfloat16, lo, hi)
    def permutation(self, n):
        return jax.random.permutation(self._next(), n)


kernel_name = 'concat_heads__spectral_gfnet__sliding_block__prompt'

def setup_inputs():
    _rng = _Rng(jax.random.key(int.from_bytes(__import__("os").urandom(4), "little")))
    _w = (lambda a: (lambda t: t.astype(jnp.bfloat16) if jnp.issubdtype(t.dtype, jnp.floating) else t)(jnp.asarray(a)))
    def _A_setup():
        B, S, D = 1, 2048, 640
        Df = D // 2 + 1
        return {
            "x": _w((lambda *s: _rng.normal(s) * 0.05)(B, S, D)),
            "w_r": _w((lambda *s: _rng.normal(s) * 0.4)(S, Df) * 0.02),
            "w_i": _w((lambda *s: _rng.normal(s) * 0.4)(S, Df) * 0.02),
        }
    _A_in = _A_setup()

    def _B_setup():
        B, S, D = 1, 2048, 640
        return {
            "x": _w((lambda *s: _rng.normal(s) * 0.2)(B, S, D)),
            "wqkv": _w((lambda *s: _rng.normal(s) * 0.2)(D, 3 * D)),
            "wo": _w((lambda *s: _rng.normal(s) * 0.05)(D, D)),
        }
    _B_in = _B_setup()

    return {
        "A_x": _A_in["x"],
        "A_w_r": _A_in["w_r"],
        "A_w_i": _A_in["w_i"],
        "B_x": _B_in["x"],
        "B_wqkv": _B_in["wqkv"],
        "B_wo": _B_in["wo"],
    }

def reference(A_x, A_w_r, A_w_i, B_x, B_wqkv, B_wo):
    def _A_ref(x, w_r, w_i):
        B, S, D = x.shape
        X = (lambda x, axes=(-2,-1): jnp.fft.rfft2(x.astype(jnp.float32), axes=axes))(x, axes=(-2, -1))
        W = w_r + 1j * w_i
        X = X * W
        y = (lambda x, s, axes=(-2,-1): jnp.fft.irfft2(x, s=s, axes=axes).astype(jnp.bfloat16))(X, (S, D), axes=(-2, -1))
        return y

    def _B_ref(x, wqkv, wo):
        B, S, D = x.shape
        H = 32; Dh = D // H; W = 256
        qkv = (lambda x, *d: x.transpose(*d))((x @ wqkv).reshape(B, S, 3, H, Dh), 2, 0, 3, 1, 4)
        q, k, v = qkv[0], qkv[1], qkv[2]
        scores = jnp.einsum("bhqd,bhkd->bhqk", q, k) * (Dh ** -0.5)
        idx = jnp.arange(S)
        mask = (idx[:, None] - idx[None, :] >= 0) & (idx[:, None] - idx[None, :] < W)
        scores = jnp.where(mask[None, None], scores, -1e9)
        p = _softmax(scores, axis=-1)
        o = jnp.einsum("bhqk,bhkd->bhqd", p, v)
        return (lambda x, *d: x.transpose(*d))(o, 0, 2, 1, 3).reshape(B, S, D) @ wo

    a = _A_ref(A_x, A_w_r, A_w_i)
    b = _B_ref(B_x, B_wqkv, B_wo)
    return jnp.concatenate([a, b], axis=-1)
```

```python
import functools
import math

import numpy as np
import jax
import jax.numpy as jnp
from jax import lax
import jax.experimental.pallas as pl
import jax.experimental.pallas.tpu as pltpu

S = 2048
D = 640
DF = D // 2 + 1
CP = 384
H = 32
DH = D // H
WIN = 256
N1 = 16
N2 = 128
RB = 256
NB = S // RB
TQ = 128
KS = TQ + WIN
NW = D // 128


def _window_heads():
    out = []
    for j in range(NW):
        lst = []
        for h in range(H):
            lo = max(DH * h, 128 * j)
            hi = min(DH * h + DH, 128 * j + 128)
            if hi > lo:
                lst.append((h, lo - 128 * j, hi - 128 * j))
        out.append(lst)
    return out


_WINDOW_HEADS = _window_heads()


@functools.lru_cache(maxsize=None)
def _dft_constants():
    d = np.arange(D)[:, None].astype(np.float64)
    k = np.arange(DF)[None, :].astype(np.float64)
    ang = 2.0 * np.pi * ((d * k) % D) / D
    fd = np.zeros((D, 2 * CP), np.float64)
    fd[:, :DF] = np.cos(ang)
    fd[:, CP:CP + DF] = -np.sin(ang)
    c = np.full((DF,), 2.0)
    c[0] = 1.0
    c[DF - 1] = 1.0
    fdi = np.zeros((2 * CP, D), np.float64)
    fdi[:DF, :] = (c[:, None] * np.cos(ang.T)) / (S * D)
    sn = -(c[:, None] * np.sin(ang.T)) / (S * D)
    sn[0, :] = 0.0
    sn[DF - 1, :] = 0.0
    fdi[CP:CP + DF, :] = sn
    g = np.zeros((N1, 2 * N2, 2 * N2), np.float64)
    gi = np.zeros((N1, 2 * N2, 2 * N2), np.float64)
    k2 = np.arange(N2)[:, None]
    s2 = np.arange(N2)[None, :]
    for k1 in range(N1):
        a = 2.0 * np.pi * ((s2 * (N1 * k2 + k1)) % S) / S
        gr = np.cos(a)
        gim = -np.sin(a)
        g[k1, :N2, :N2] = gr
        g[k1, :N2, N2:] = -gim
        g[k1, N2:, :N2] = gim
        g[k1, N2:, N2:] = gr
        gi[k1, :N2, :N2] = gr.T
        gi[k1, :N2, N2:] = gim.T
        gi[k1, N2:, :N2] = -gim.T
        gi[k1, N2:, N2:] = gr.T
    bf = jnp.bfloat16
    return (np.asarray(fd, np.float32).astype(bf), np.asarray(fdi, np.float32).astype(bf),
            np.asarray(g, np.float32).astype(bf), np.asarray(gi, np.float32).astype(bf))


def _cmul_const(xr, xi, ang):
    c = math.cos(ang)
    s = math.sin(ang)
    eps = 1e-12
    if abs(s) < eps:
        return (xr, xi) if c > 0 else (-xr, -xi)
    if abs(c) < eps:
        return (-xi, xr) if s > 0 else (xi, -xr)
    if abs(abs(c) - abs(s)) < eps:
        r = abs(c)
        if c > 0 and s > 0:
            return (xr - xi) * r, (xr + xi) * r
        if c > 0 and s < 0:
            return (xr + xi) * r, (xi - xr) * r
        if c < 0 and s > 0:
            return (-xr - xi) * r, (xr - xi) * r
        return (xi - xr) * r, (-xr - xi) * r
    return xr * c - xi * s, xr * s + xi * c


def _dft4(x, sign):
    (ar, ai), (br, bi), (cr, ci), (dr, di) = x
    s0r, s0i = ar + cr, ai + ci
    s1r, s1i = ar - cr, ai - ci
    s2r, s2i = br + dr, bi + di
    s3r, s3i = br - dr, bi - di
    y0 = (s0r + s2r, s0i + s2i)
    y2 = (s0r - s2r, s0i - s2i)
    if sign < 0:
        tr, ti = s3i, -s3r
    else:
        tr, ti = -s3i, s3r
    y1 = (s1r + tr, s1i + ti)
    y3 = (s1r - tr, s1i - ti)
    return [y0, y1, y2, y3]


def _dft16(x, sign):
    t = []
    for b in range(4):
        col = _dft4([x[4 * a + b] for a in range(4)], sign)
        col = [_cmul_const(col[c][0], col[c][1], sign * 2.0 * math.pi * b * c / 16.0)
               for c in range(4)]
        t.append(col)
    out = [None] * 16
    for c in range(4):
        row = _dft4([t[b][c] for b in range(4)], sign)
        for d in range(4):
            out[c + 4 * d] = row[d]
    return out


def _radix16_pass(u_ref, sign):
    def body(r, carry):
        r0 = pl.multiple_of(r * 8, 8)
        for l in range(CP // 128):
            xs = []
            for b in range(N1):
                re = u_ref[pl.ds(b * N2 + r0, 8), pl.ds(l * 128, 128)]
                im = u_ref[pl.ds(b * N2 + r0, 8), pl.ds(CP + l * 128, 128)]
                xs.append((re, im))
            ys = _dft16(xs, sign)
            for b in range(N1):
                u_ref[pl.ds(b * N2 + r0, 8), pl.ds(l * 128, 128)] = ys[b][0]
                u_ref[pl.ds(b * N2 + r0, 8), pl.ds(CP + l * 128, 128)] = ys[b][1]
        return carry
    lax.fori_loop(0, N2 // 8, body, 0)


def _kernel(xa_ref, wrt_ref, wit_ref, xb_ref, wqkv_hbm, wo_hbm,
            fd_hbm, fdi_hbm, g_hbm, gi_hbm,
            o_ref,
            u_ref, k_ref, vt_ref, wvt_ref, ot_ref,
            wqkv_ref, wo_ref, fd_ref, fdi_ref, g_ref, gi_ref,
            wf_ref, sems):
    t = pl.program_id(0)
    f32 = jnp.float32
    bf16 = jnp.bfloat16
    NT = (((1,), (1,)), ((), ()))

    copies = [
        pltpu.make_async_copy(fd_hbm, fd_ref, sems.at[0]),
        pltpu.make_async_copy(wqkv_hbm, wqkv_ref, sems.at[1]),
        pltpu.make_async_copy(wo_hbm, wo_ref, sems.at[2]),
        pltpu.make_async_copy(g_hbm, g_ref, sems.at[3]),
        pltpu.make_async_copy(gi_hbm, gi_ref, sems.at[4]),
        pltpu.make_async_copy(fdi_hbm, fdi_ref, sems.at[5]),
    ]

    @pl.when(t == 0)
    def _():
        for c in copies:
            c.start()
        k_ref[pl.ds(0, WIN), :] = jnp.zeros((WIN, D), bf16)
        vt_ref[:, pl.ds(0, WIN)] = jnp.zeros((D, WIN), bf16)
        copies[0].wait()

    def phase1(first):
        r0 = pl.multiple_of(t * RB, RB)
        u_ref[pl.ds(r0, RB), :] = jnp.dot(xa_ref[...], fd_ref[...],
                                          preferred_element_type=f32)
        for i, w_ref in enumerate((wrt_ref, wit_ref)):
            for b in range(RB // 128):
                for l in range(3):
                    nr = min(128, DF - 128 * l)
                    tile = w_ref[pl.ds(128 * l, nr), pl.ds(128 * b, 128)].astype(f32)
                    if nr < 128:
                        tile = jnp.concatenate(
                            [tile, jnp.zeros((128 - nr, 128), f32)], axis=0)
                    wf_ref[3 * i + l, pl.ds(r0 + 128 * b, 128), :] = tile.T

        if first:
            copies[1].wait()
            copies[2].wait()
            wvt_ref[...] = wqkv_ref[:, pl.ds(2 * D, D)].astype(f32).T.astype(bf16)

        xb = xb_ref[...]
        qk = jnp.dot(xb, wqkv_ref[:, pl.ds(0, 2 * D)], preferred_element_type=f32)
        q_all = (qk[:, :D] * (DH ** -0.5)).astype(bf16)
        k_ref[pl.ds(WIN + r0, RB), :] = qk[:, D:].astype(bf16)
        vt_ref[:, pl.ds(WIN + r0, RB)] = lax.dot_general(
            wvt_ref[...], xb, NT, preferred_element_type=f32).astype(bf16)

        lane = lax.broadcasted_iota(jnp.int32, (1, 128), 1)
        jj = lax.broadcasted_iota(jnp.int32, (TQ, TQ), 0)
        ii = lax.broadcasted_iota(jnp.int32, (TQ, TQ), 1)
        upper = jj > ii
        lower = jj <= ii
        row32 = lax.broadcasted_iota(jnp.int32, (32, TQ), 0)
        NEG = -1e30

        units = [(u, j) for u in range(RB // TQ) for j in range(NW)]

        def qk_scores(u, j):
            q0 = pl.multiple_of(r0 + u * TQ, TQ)
            heads = _WINDOW_HEADS[j]
            qw = q_all[u * TQ:(u + 1) * TQ, 128 * j:128 * (j + 1)]
            kw = k_ref[pl.ds(q0, KS), pl.ds(128 * j, 128)]
            qm = jnp.concatenate(
                [jnp.where((lane >= lo) & (lane < hi), qw, jnp.zeros_like(qw))
                 for (_, lo, hi) in heads], axis=0)
            return lax.dot_general(kw, qm, NT, preferred_element_type=f32)

        carry = [None]

        def finish(u, j, s_all):
            q0 = pl.multiple_of(r0 + u * TQ, TQ)
            heads = _WINDOW_HEADS[j]
            parts = [s_all[:, i * TQ:(i + 1) * TQ] for i in range(len(heads))]
            if DH * heads[0][0] < 128 * j:
                parts[0] = parts[0] + carry[0]
            if DH * heads[-1][0] + DH > 128 * (j + 1):
                carry[0] = parts[-1]
                parts = parts[:-1]
                done = heads[:-1]
            else:
                done = heads
            for i, (h, lo, hi) in enumerate(done):
                s = parts[i]
                s0, s1, s2 = s[:TQ], s[TQ:2 * TQ], s[2 * TQ:]
                s2 = jnp.where(lower, s2, NEG)
                if first:
                    if u == 0:
                        blocks = [s2]
                        kofs = 2 * TQ
                    else:
                        blocks = [s1, s2]
                        kofs = TQ
                else:
                    s0 = jnp.where(upper, s0, NEG)
                    blocks = [s0, s1, s2]
                    kofs = 0
                nk = len(blocks) * TQ
                sm = blocks[0]
                for b in blocks[1:]:
                    sm = jnp.maximum(sm, b)
                m = jnp.max(sm, axis=0, keepdims=True)
                pb = jnp.concatenate(
                    [jnp.exp(b - m).astype(bf16) for b in blocks], axis=0)
                a = (DH * h // 16) * 16
                off = DH * h - a
                spare = off + DH if off + DH < 32 else 0
                vt = vt_ref[pl.ds(a, 32), pl.ds(q0 + kofs, nk)]
                vt = jnp.where(lax.broadcasted_iota(jnp.int32, (32, nk), 0) == spare,
                               jnp.ones_like(vt), vt)
                oh = jnp.dot(vt, pb, preferred_element_type=f32)
                inv_l = 1.0 / oh[spare:spare + 1, :]
                rmask = (row32 >= off) & (row32 < off + DH)
                if h == 0:
                    ot_ref[pl.ds(a, 32), :] = jnp.where(rmask, oh * inv_l, 0.0)
                else:
                    ot_ref[pl.ds(a, 32), :] = jnp.where(
                        rmask, oh * inv_l, ot_ref[pl.ds(a, 32), :])
            if j == NW - 1:
                ot = ot_ref[...].astype(bf16)
                o_ref[pl.ds(u * TQ, TQ), :] = lax.dot_general(
                    ot, wo_ref[...], (((0,), (0,)), ((), ())),
                    preferred_element_type=f32).astype(o_ref.dtype)

        s_cur = qk_scores(*units[0])
        for n, (u, j) in enumerate(units):
            s_next = qk_scores(*units[n + 1]) if n + 1 < len(units) else None
            finish(u, j, s_cur)
            s_cur = s_next

    @pl.when(t == 0)
    def _():
        phase1(True)

    @pl.when((t > 0) & (t < NB))
    def _():
        phase1(False)

    @pl.when(t == NB)
    def _phase2():
        for c in copies[3:]:
            c.wait()
        _radix16_pass(u_ref, -1)

        def body(k1, carry):
            r0 = pl.multiple_of(k1 * N2, N2)
            blk = u_ref[pl.ds(r0, N2), :]
            st = jnp.concatenate([blk[:, :CP], blk[:, CP:]], axis=0).astype(bf16)
            z = jnp.dot(g_ref[k1], st, preferred_element_type=f32)
            zr = z[:N2]
            zi = z[N2:]
            wr = jnp.concatenate(
                [wf_ref[l, pl.ds(k1, N2, stride=N1), :] for l in range(3)], axis=1)
            wi = jnp.concatenate(
                [wf_ref[3 + l, pl.ds(k1, N2, stride=N1), :] for l in range(3)], axis=1)
            yr = zr * wr - zi * wi
            yi = zr * wi + zi * wr
            yst = jnp.concatenate([yr, yi], axis=0).astype(bf16)
            v = jnp.dot(gi_ref[k1], yst, preferred_element_type=f32)
            u_ref[pl.ds(r0, N2), pl.ds(0, CP)] = v[:N2]
            u_ref[pl.ds(r0, N2), pl.ds(CP, CP)] = v[N2:]
            return carry
        lax.fori_loop(0, N1, body, 0)

        _radix16_pass(u_ref, +1)

    @pl.when(t >= NB)
    def _phase3():
        r0 = pl.multiple_of((t - NB) * RB, RB)
        ub = u_ref[pl.ds(r0, RB), :].astype(bf16)
        o_ref[...] = jnp.dot(ub, fdi_ref[...],
                             preferred_element_type=f32).astype(o_ref.dtype)


@jax.jit
def pallas_concat_heads__spectral_gfnet__sliding_block__prompt_kernel(
    A_x: jax.Array,
    A_w_r: jax.Array,
    A_w_i: jax.Array,
    B_x: jax.Array,
    B_wqkv: jax.Array,
    B_wo: jax.Array,
):
    bf16 = jnp.bfloat16
    fd, fdi, g, gi = _dft_constants()
    xa = A_x.reshape(S, D)
    xb = B_x.reshape(S, D)

    row_spec = pl.BlockSpec((RB, D), lambda t: (jnp.minimum(t, NB - 1), 0))
    any_spec = pl.BlockSpec(memory_space=pl.ANY)
    wt_spec = pl.BlockSpec((DF, RB), lambda t: (0, jnp.minimum(t, NB - 1)))

    out = pl.pallas_call(
        _kernel,
        grid=(2 * NB,),
        in_specs=[row_spec, wt_spec, wt_spec, row_spec, any_spec, any_spec,
                  any_spec, any_spec, any_spec, any_spec],
        out_specs=pl.BlockSpec(
            (RB, D), lambda t: (jnp.where(t < NB, t, t - NB), jnp.where(t < NB, 1, 0))),
        out_shape=jax.ShapeDtypeStruct((S, 2 * D), bf16),
        scratch_shapes=[
            pltpu.VMEM((S, 2 * CP), jnp.float32),
            pltpu.VMEM((S + WIN, D), bf16),
            pltpu.VMEM((D, S + WIN), bf16),
            pltpu.VMEM((D, D), bf16),
            pltpu.VMEM((D, TQ), jnp.float32),
            pltpu.VMEM((D, 3 * D), bf16),
            pltpu.VMEM((D, D), bf16),
            pltpu.VMEM((D, 2 * CP), bf16),
            pltpu.VMEM((2 * CP, D), bf16),
            pltpu.VMEM((N1, 2 * N2, 2 * N2), bf16),
            pltpu.VMEM((N1, 2 * N2, 2 * N2), bf16),
            pltpu.VMEM((6, S, 128), jnp.float32),
            pltpu.SemaphoreType.DMA((6,)),
        ],
        compiler_params=pltpu.CompilerParams(
            dimension_semantics=("arbitrary",),
            vmem_limit_bytes=126 * 1024 * 1024,
        ),
    )(xa, A_w_r.T, A_w_i.T, xb, B_wqkv, B_wo, fd, fdi, g, gi)
    return out.reshape(1, S, 2 * D)
```

```python
import functools
import math

import numpy as np
import jax
import jax.numpy as jnp
from jax import lax
import jax.experimental.pallas as pl
import jax.experimental.pallas.tpu as pltpu

S = 2048
D = 640
DF = D // 2 + 1
CP = 384
H = 32
DH = D // H
WIN = 256
N1 = 16
N2 = 128
RB = 256
NB = S // RB
TQ = 128
KS = TQ + WIN
NW = D // 128


def _window_heads():
    out = []
    for j in range(NW):
        lst = []
        for h in range(H):
            lo = max(DH * h, 128 * j)
            hi = min(DH * h + DH, 128 * j + 128)
            if hi > lo:
                lst.append((h, lo - 128 * j, hi - 128 * j))
        out.append(lst)
    return out


_WINDOW_HEADS_ALL = _window_heads()
_WINDOW_HEADS = [[(h, lo, hi) for (h, lo, hi) in lst if hi - lo == DH]
                 for lst in _WINDOW_HEADS_ALL]
_STRADDLE = [(h, w, DH * h - (128 * w + 64), DH * h + DH - (128 * w + 64))
             for w in range(NW - 1) for h in range(H)
             if DH * h < 128 * (w + 1) < DH * h + DH]
_C1 = math.cos(2.0 * math.pi / 5.0)
_C2 = math.cos(4.0 * math.pi / 5.0)
_S1 = math.sin(2.0 * math.pi / 5.0)
_S2 = math.sin(4.0 * math.pi / 5.0)


def _class_freqs():
    c0 = [5 * m for m in range(65)] + [None] * 63
    c1 = [1 + 5 * m for m in range(64)] + [4 + 5 * m for m in range(64)]
    c2 = [2 + 5 * m for m in range(64)] + [3 + 5 * m for m in range(64)]
    return [c0, c1, c2]


@functools.lru_cache(maxsize=None)
def _dft_constants():
    freqs = _class_freqs()
    d2 = np.arange(128).astype(np.float64)
    norm = 1.0 / (S * D)
    fd = np.zeros((640, 256), np.float64)
    fdi = np.zeros((256, 640), np.float64)
    for lane, k in enumerate(freqs[0]):
        if k is None:
            continue
        th = 2.0 * np.pi * ((d2 * k) % D) / D
        sn = np.sin(th)
        if k == 0 or k == DF - 1:
            sn = np.zeros_like(sn)
        fd[0:128, lane] = np.cos(th)
        fd[0:128, 128 + lane] = -sn
        ck = 1.0 if (k == 0 or k == DF - 1) else 2.0
        fdi[lane, 0:128] = ck * np.cos(th) * norm
        fdi[128 + lane, 0:128] = -ck * sn * norm
    for c in (1, 2):
        rb = 128 + 256 * (c - 1)
        for lane, k in enumerate(freqs[c]):
            th = 2.0 * np.pi * ((d2 * k) % D) / D
            cs, sn = np.cos(th), np.sin(th)
            sg = 1.0 if (k % 5) == c else -1.0
            fd[rb:rb + 128, lane] = cs
            fd[rb + 128:rb + 256, lane] = sg * sn
            fd[rb:rb + 128, 128 + lane] = -sn
            fd[rb + 128:rb + 256, 128 + lane] = sg * cs
            fdi[lane, rb:rb + 128] = 2.0 * cs * norm
            fdi[128 + lane, rb:rb + 128] = -2.0 * sn * norm
            fdi[lane, rb + 128:rb + 256] = sg * 2.0 * sn * norm
            fdi[128 + lane, rb + 128:rb + 256] = sg * 2.0 * cs * norm
    g = np.zeros((N1, 2 * N2, 2 * N2), np.float64)
    gi = np.zeros((N1, 2 * N2, 2 * N2), np.float64)
    k2 = np.arange(N2)[:, None]
    s2 = np.arange(N2)[None, :]
    for k1 in range(N1):
        a = 2.0 * np.pi * ((s2 * (N1 * k2 + k1)) % S) / S
        gr = np.cos(a)
        gim = -np.sin(a)
        g[k1, :N2, :N2] = gr
        g[k1, :N2, N2:] = -gim
        g[k1, N2:, :N2] = gim
        g[k1, N2:, N2:] = gr
        gi[k1, :N2, :N2] = gr.T
        gi[k1, :N2, N2:] = gim.T
        gi[k1, N2:, :N2] = -gim.T
        gi[k1, N2:, N2:] = gr.T
    bf = jnp.bfloat16
    return (np.asarray(fd, np.float32).astype(bf), np.asarray(fdi, np.float32).astype(bf),
            np.asarray(g, np.float32).astype(bf), np.asarray(gi, np.float32).astype(bf))


def _cmul_const(xr, xi, ang):
    c = math.cos(ang)
    s = math.sin(ang)
    eps = 1e-12
    if abs(s) < eps:
        return (xr, xi) if c > 0 else (-xr, -xi)
    if abs(c) < eps:
        return (-xi, xr) if s > 0 else (xi, -xr)
    if abs(abs(c) - abs(s)) < eps:
        r = abs(c)
        if c > 0 and s > 0:
            return (xr - xi) * r, (xr + xi) * r
        if c > 0 and s < 0:
            return (xr + xi) * r, (xi - xr) * r
        if c < 0 and s > 0:
            return (-xr - xi) * r, (xr - xi) * r
        return (xi - xr) * r, (-xr - xi) * r
    return xr * c - xi * s, xr * s + xi * c


def _dft4(x, sign):
    (ar, ai), (br, bi), (cr, ci), (dr, di) = x
    s0r, s0i = ar + cr, ai + ci
    s1r, s1i = ar - cr, ai - ci
    s2r, s2i = br + dr, bi + di
    s3r, s3i = br - dr, bi - di
    y0 = (s0r + s2r, s0i + s2i)
    y2 = (s0r - s2r, s0i - s2i)
    if sign < 0:
        tr, ti = s3i, -s3r
    else:
        tr, ti = -s3i, s3r
    y1 = (s1r + tr, s1i + ti)
    y3 = (s1r - tr, s1i - ti)
    return [y0, y1, y2, y3]


def _dft16(x, sign):
    t = []
    for b in range(4):
        col = _dft4([x[4 * a + b] for a in range(4)], sign)
        col = [_cmul_const(col[c][0], col[c][1], sign * 2.0 * math.pi * b * c / 16.0)
               for c in range(4)]
        t.append(col)
    out = [None] * 16
    for c in range(4):
        row = _dft4([t[b][c] for b in range(4)], sign)
        for d in range(4):
            out[c + 4 * d] = row[d]
    return out


def _radix16_pass(u_ref, sign):
    def body(r, carry):
        r0 = pl.multiple_of(r * 8, 8)
        for l in range(CP // 128):
            xs = []
            for b in range(N1):
                re = u_ref[pl.ds(b * N2 + r0, 8), pl.ds(l * 128, 128)]
                im = u_ref[pl.ds(b * N2 + r0, 8), pl.ds(CP + l * 128, 128)]
                xs.append((re, im))
            ys = _dft16(xs, sign)
            for b in range(N1):
                u_ref[pl.ds(b * N2 + r0, 8), pl.ds(l * 128, 128)] = ys[b][0]
                u_ref[pl.ds(b * N2 + r0, 8), pl.ds(CP + l * 128, 128)] = ys[b][1]
        return carry
    lax.fori_loop(0, N2 // 8, body, 0)


def _kernel(xa_ref, wrt_ref, wit_ref, xb_ref, wqkv_hbm, wo_hbm,
            fd_hbm, fdi_hbm, g_hbm, gi_hbm,
            out_hbm,
            u_ref, k_ref, k2_ref, vt_ref, wvt_ref, ot_ref,
            ob_ref, oa_ref, y0_ref, y1_ref, osems, asems,
            wqkv_ref, wo_ref, fd_ref, fdi_ref, g_ref, gi_ref,
            wf_ref, wtmp_ref, sems):
    t = pl.program_id(0)
    f32 = jnp.float32
    bf16 = jnp.bfloat16
    NT = (((1,), (1,)), ((), ()))

    copies = [
        pltpu.make_async_copy(fd_hbm, fd_ref, sems.at[0]),
        pltpu.make_async_copy(wqkv_hbm, wqkv_ref, sems.at[1]),
        pltpu.make_async_copy(wo_hbm, wo_ref, sems.at[2]),
        pltpu.make_async_copy(g_hbm, g_ref, sems.at[3]),
        pltpu.make_async_copy(gi_hbm, gi_ref, sems.at[4]),
        pltpu.make_async_copy(fdi_hbm, fdi_ref, sems.at[5]),
    ]

    @pl.when(t == 0)
    def _():
        for c in copies:
            c.start()
        k_ref[pl.ds(0, WIN), :] = jnp.zeros((WIN, D), bf16)
        k2_ref[pl.ds(0, WIN), :] = jnp.zeros((WIN, D - 128), bf16)
        ot_ref[...] = jnp.zeros((D, TQ), f32)
        vt_ref[:, pl.ds(0, WIN)] = jnp.zeros((D, WIN), bf16)
        copies[0].wait()

    def b_copy(step, slot):
        return pltpu.make_async_copy(
            ob_ref.at[slot],
            out_hbm.at[pl.ds(step * (RB // N2), RB // N2), :, pl.ds(D, D)],
            osems.at[slot])

    def phase1(first):
        r0 = pl.multiple_of(t * RB, RB)
        slot = t % 2
        if not first:
            @pl.when(t >= 2)
            def _():
                b_copy(t - 2, slot).wait()
        x5 = [xa_ref[:, pl.ds(128 * i, 128)].astype(f32) for i in range(5)]
        t1 = x5[1] + x5[4]
        t2 = x5[2] + x5[3]
        t3 = x5[1] - x5[4]
        t4 = x5[2] - x5[3]
        a0 = x5[0] + t1 + t2
        a1r = x5[0] + _C1 * t1 + _C2 * t2
        a1i = -(_S1 * t3 + _S2 * t4)
        a2r = x5[0] + _C2 * t1 + _C1 * t2
        a2i = -(_S2 * t3 - _S1 * t4)
        ins = [a0.astype(bf16),
               jnp.concatenate([a1r, a1i], axis=1).astype(bf16),
               jnp.concatenate([a2r, a2i], axis=1).astype(bf16)]
        for c in range(3):
            m_lo, m_n = (0, 128) if c == 0 else (128 + 256 * (c - 1), 256)
            uc = jnp.dot(ins[c], fd_ref[pl.ds(m_lo, m_n), :],
                         preferred_element_type=f32)
            u_ref[pl.ds(r0, RB), pl.ds(128 * c, 128)] = uc[:, :128]
            u_ref[pl.ds(r0, RB), pl.ds(CP + 128 * c, 128)] = uc[:, 128:]
        for i, w_ref in enumerate((wrt_ref, wit_ref)):
            for b in range(RB // 128):
                wtmp_ref[b, pl.ds(0, DF), :] = (
                    w_ref[:, pl.ds(128 * b, 128)].astype(f32))
                def rows(c, n, _b=b):
                    return wtmp_ref[_b, pl.ds(c, n, stride=5), :]
                tiles = [
                    jnp.concatenate([rows(0, 65), jnp.zeros((63, 128), f32)], axis=0),
                    jnp.concatenate([rows(1, 64), rows(4, 64)], axis=0),
                    jnp.concatenate([rows(2, 64), rows(3, 64)], axis=0),
                ]
                for l in range(3):
                    wf_ref[3 * i + l, pl.ds(r0 + 128 * b, 128), :] = tiles[l].T

        if first:
            copies[1].wait()
            copies[2].wait()
            wvt_ref[...] = wqkv_ref[:, pl.ds(2 * D, D)].astype(f32).T.astype(bf16)

        xb = xb_ref[...]
        qk = jnp.dot(xb, wqkv_ref[:, pl.ds(0, 2 * D)], preferred_element_type=f32)
        q_all = (qk[:, :D] * (DH ** -0.5 * math.log2(math.e))).astype(bf16)
        k_ref[pl.ds(WIN + r0, RB), :] = qk[:, D:].astype(bf16)
        k2_ref[pl.ds(WIN + r0, RB), :] = qk[:, D + 64:2 * D - 64].astype(bf16)
        q2_all = (qk[:, 64:D - 64] * (DH ** -0.5 * math.log2(math.e))).astype(bf16)
        vt_ref[:, pl.ds(WIN + r0, RB)] = lax.dot_general(
            wvt_ref[...], xb, NT, preferred_element_type=f32).astype(bf16)

        lane = lax.broadcasted_iota(jnp.int32, (1, 128), 1)
        jj = lax.broadcasted_iota(jnp.int32, (TQ, TQ), 0)
        ii = lax.broadcasted_iota(jnp.int32, (TQ, TQ), 1)
        upper = jj > ii
        lower = jj <= ii
        row32 = lax.broadcasted_iota(jnp.int32, (32, TQ), 0)
        NEG = -1e30

        units = [(u, j) for u in range(RB // TQ) for j in range(NW + 1)]

        def qk_scores(u, j):
            q0 = pl.multiple_of(r0 + u * TQ, TQ)
            if j == 0:
                outs = []
                for (h, w, lo, hi) in _STRADDLE:
                    qw = q2_all[u * TQ:(u + 1) * TQ, 128 * w:128 * (w + 1)]
                    kw = k2_ref[pl.ds(q0, KS), pl.ds(128 * w, 128)]
                    qm = jnp.where((lane >= lo) & (lane < hi), qw, jnp.zeros_like(qw))
                    outs.append(lax.dot_general(kw, qm, NT,
                                                preferred_element_type=f32))
                return jnp.concatenate(outs, axis=1)
            j = j - 1
            heads = _WINDOW_HEADS[j]
            qw = q_all[u * TQ:(u + 1) * TQ, 128 * j:128 * (j + 1)]
            kw = k_ref[pl.ds(q0, KS), pl.ds(128 * j, 128)]
            qm = jnp.concatenate(
                [jnp.where((lane >= lo) & (lane < hi), qw, jnp.zeros_like(qw))
                 for (_, lo, hi) in heads], axis=0)
            return lax.dot_general(kw, qm, NT, preferred_element_type=f32)

        def finish(u, j, s_all):
            q0 = pl.multiple_of(r0 + u * TQ, TQ)
            done = _STRADDLE if j == 0 else _WINDOW_HEADS[j - 1]
            parts = [s_all[:, i * TQ:(i + 1) * TQ] for i in range(len(done))]
            for i, hd in enumerate(done):
                h = hd[0]
                s = parts[i]
                s0, s1, s2 = s[:TQ], s[TQ:2 * TQ], s[2 * TQ:]
                if first:
                    s2 = jnp.where(lower, s2, NEG)
                    if u == 0:
                        blocks = [s2]
                        kofs = 2 * TQ
                    else:
                        blocks = [s1, s2]
                        kofs = TQ
                    nk = len(blocks) * TQ
                    sm = blocks[0]
                    for b in blocks[1:]:
                        sm = jnp.maximum(sm, b)
                    m = jnp.max(sm, axis=0, keepdims=True)
                    pb = jnp.concatenate(
                        [jnp.exp2(b - m).astype(bf16) for b in blocks], axis=0)
                else:
                    sx = jnp.where(lower, s2, s0)
                    kofs = 0
                    nk = KS
                    m = jnp.max(jnp.maximum(sx, s1), axis=0, keepdims=True)
                    px = jnp.exp2(sx - m).astype(bf16)
                    p1 = jnp.exp2(s1 - m).astype(bf16)
                    zero = jnp.zeros_like(px)
                    pb = jnp.concatenate(
                        [jnp.where(lower, zero, px), p1, jnp.where(lower, px, zero)],
                        axis=0)
                a = (DH * h // 16) * 16
                off = DH * h - a
                spare = off + DH if off + DH < 32 else 0
                vt = vt_ref[pl.ds(a, 32), pl.ds(q0 + kofs, nk)]
                vt = jnp.where(lax.broadcasted_iota(jnp.int32, (32, nk), 0) == spare,
                               jnp.ones_like(vt), vt)
                oh = jnp.dot(vt, pb, preferred_element_type=f32)
                inv_l = 1.0 / oh[spare:spare + 1, :]
                rmask = (row32 >= off) & (row32 < off + DH)
                ot_ref[pl.ds(a, 32), :] = jnp.where(
                    rmask, oh * inv_l, ot_ref[pl.ds(a, 32), :])
            if j == NW:
                ot = ot_ref[...].astype(bf16)
                ob_ref[slot, u] = lax.dot_general(
                    ot, wo_ref[...], (((0,), (0,)), ((), ())),
                    preferred_element_type=f32).astype(bf16)

        s_cur = qk_scores(*units[0])
        for n, (u, j) in enumerate(units):
            s_next = qk_scores(*units[n + 1]) if n + 1 < len(units) else None
            finish(u, j, s_cur)
            s_cur = s_next
        b_copy(t, slot).start()

    @pl.when(t == 0)
    def _():
        phase1(True)

    @pl.when(t > 0)
    def _():
        phase1(False)

    @pl.when(t == NB - 1)
    def _phase2():
        for c in copies[3:]:
            c.wait()
        _radix16_pass(u_ref, -1)

        NP = 4

        def body(kk, carry):
            ks = [kk * NP + i for i in range(NP)]
            r0s = [pl.multiple_of(k1 * N2, N2) for k1 in ks]
            sts = []
            for r0 in r0s:
                blk = u_ref[pl.ds(r0, N2), :]
                sts.append(jnp.concatenate([blk[:, :CP], blk[:, CP:]],
                                           axis=0).astype(bf16))
            zs = [jnp.dot(g_ref[k1], st, preferred_element_type=f32)
                  for k1, st in zip(ks, sts)]
            vs = []
            for k1, z in zip(ks, zs):
                zr = z[:N2]
                zi = z[N2:]
                wr = jnp.concatenate(
                    [wf_ref[l, pl.ds(k1, N2, stride=N1), :] for l in range(3)], axis=1)
                wi = jnp.concatenate(
                    [wf_ref[3 + l, pl.ds(k1, N2, stride=N1), :] for l in range(3)],
                    axis=1)
                yr = zr * wr - zi * wi
                yi = zr * wi + zi * wr
                yst = jnp.concatenate([yr, yi], axis=0).astype(bf16)
                vs.append(jnp.dot(gi_ref[k1], yst, preferred_element_type=f32))
            for r0, v in zip(r0s, vs):
                u_ref[pl.ds(r0, N2), pl.ds(0, CP)] = v[:N2]
                u_ref[pl.ds(r0, N2), pl.ds(CP, CP)] = v[N2:]
            return carry
        lax.fori_loop(0, N1 // NP, body, 0)

        def inv_radix(r, y_ref):
            for sub in range(2):
                rr = pl.multiple_of(r * 16 + sub * 8, 8)
                for l in range(CP // 128):
                    xs = []
                    for b in range(N1):
                        re = u_ref[pl.ds(b * N2 + rr, 8), pl.ds(l * 128, 128)]
                        im = u_ref[pl.ds(b * N2 + rr, 8), pl.ds(CP + l * 128, 128)]
                        xs.append((re, im))
                    ys = _dft16(xs, +1)
                    for b in range(N1):
                        y_ref[pl.ds(b * 16 + sub * 8, 8), pl.ds(256 * l, 128)] = ys[b][0]
                        y_ref[pl.ds(b * 16 + sub * 8, 8),
                              pl.ds(256 * l + 128, 128)] = ys[b][1]

        def inv_d(r, y_ref):
            cs = []
            for c in range(3):
                yc = y_ref[:, pl.ds(256 * c, 256)].astype(bf16)
                m_lo, m_n = (0, 128) if c == 0 else (128 + 256 * (c - 1), 256)
                cs.append(jnp.dot(yc, fdi_ref[:, pl.ds(m_lo, m_n)],
                                  preferred_element_type=f32))
            c0 = cs[0]
            c1r, c1i = cs[1][:, :128], cs[1][:, 128:]
            c2r, c2i = cs[2][:, :128], cs[2][:, 128:]
            e1 = _C1 * c1r + _C2 * c2r
            f1 = _S1 * c1i + _S2 * c2i
            e2 = _C2 * c1r + _C1 * c2r
            f2 = _S2 * c1i - _S1 * c2i
            ys = [c0 + c1r + c2r, c0 + e1 - f1, c0 + e2 - f2, c0 + e2 + f2,
                  c0 + e1 + f1]
            y = jnp.concatenate(ys, axis=1).astype(bf16)
            rr = pl.multiple_of(r * 16, 16)
            oa_ref[:, pl.ds(rr, 16), :] = y.reshape(N1, 16, D)

        def a_copy(qt):
            return pltpu.make_async_copy(
                oa_ref.at[:, pl.ds(qt * 32, 32), :],
                out_hbm.at[:, pl.ds(qt * 32, 32), pl.ds(0, D)],
                asems.at[qt])

        NR = N2 // 16
        inv_radix(0, y0_ref)
        for r in range(NR):
            cur, nxt = (y0_ref, y1_ref) if r % 2 == 0 else (y1_ref, y0_ref)
            if r + 1 < NR:
                inv_radix(r + 1, nxt)
            inv_d(r, cur)
            if r % 2 == 1:
                a_copy(r // 2).start()
        b_copy(NB - 2, (NB - 2) % 2).wait()
        b_copy(NB - 1, (NB - 1) % 2).wait()
        for qt in range(NR // 2):
            a_copy(qt).wait()


@jax.jit
def pallas_concat_heads__spectral_gfnet__sliding_block__prompt_kernel(
    A_x: jax.Array,
    A_w_r: jax.Array,
    A_w_i: jax.Array,
    B_x: jax.Array,
    B_wqkv: jax.Array,
    B_wo: jax.Array,
):
    bf16 = jnp.bfloat16
    fd, fdi, g, gi = _dft_constants()
    xa = A_x.reshape(S, D)
    xb = B_x.reshape(S, D)

    row_spec = pl.BlockSpec((RB, D), lambda t: (t, 0))
    any_spec = pl.BlockSpec(memory_space=pl.ANY)
    wt_spec = pl.BlockSpec((DF, RB), lambda t: (0, t))

    out = pl.pallas_call(
        _kernel,
        grid=(NB,),
        in_specs=[row_spec, wt_spec, wt_spec, row_spec, any_spec, any_spec,
                  any_spec, any_spec, any_spec, any_spec],
        out_specs=any_spec,
        out_shape=jax.ShapeDtypeStruct((N1, N2, 2 * D), bf16),
        scratch_shapes=[
            pltpu.VMEM((S, 2 * CP), jnp.float32),
            pltpu.VMEM((S + WIN, D), bf16),
            pltpu.VMEM((S + WIN, D - 128), bf16),
            pltpu.VMEM((D, S + WIN), bf16),
            pltpu.VMEM((D, D), bf16),
            pltpu.VMEM((D, TQ), jnp.float32),
            pltpu.VMEM((2, RB // N2, N2, D), bf16),
            pltpu.VMEM((N1, N2, D), bf16),
            pltpu.VMEM((256, 2 * CP), jnp.float32),
            pltpu.VMEM((256, 2 * CP), jnp.float32),
            pltpu.SemaphoreType.DMA((2,)),
            pltpu.SemaphoreType.DMA((4,)),
            pltpu.VMEM((D, 3 * D), bf16),
            pltpu.VMEM((D, D), bf16),
            pltpu.VMEM((D, 256), bf16),
            pltpu.VMEM((256, D), bf16),
            pltpu.VMEM((N1, 2 * N2, 2 * N2), bf16),
            pltpu.VMEM((N1, 2 * N2, 2 * N2), bf16),
            pltpu.VMEM((6, S, 128), jnp.float32),
            pltpu.VMEM((RB // 128, 328, 128), jnp.float32),
            pltpu.SemaphoreType.DMA((6,)),
        ],
        compiler_params=pltpu.CompilerParams(
            dimension_semantics=("arbitrary",),
            vmem_limit_bytes=126 * 1024 * 1024,
        ),
    )(xa, A_w_r.T, A_w_i.T, xb, B_wqkv, B_wo, fd, fdi, g, gi)
    return out.reshape(1, S, 2 * D)
```

```python
import functools
import math

import numpy as np
import jax
import jax.numpy as jnp
from jax import lax
import jax.experimental.pallas as pl
import jax.experimental.pallas.tpu as pltpu

S = 2048
D = 640
DF = D // 2 + 1
CP = 384
H = 32
DH = D // H
WIN = 256
N1 = 16
N2 = 128
RB = 256
NB = S // RB
TQ = 128
KS = TQ + WIN
NW = D // 128


def _window_heads():
    out = []
    for j in range(NW):
        lst = []
        for h in range(H):
            lo = max(DH * h, 128 * j)
            hi = min(DH * h + DH, 128 * j + 128)
            if hi > lo:
                lst.append((h, lo - 128 * j, hi - 128 * j))
        out.append(lst)
    return out


_WINDOW_HEADS_ALL = _window_heads()
_WINDOW_HEADS = [[(h, lo, hi) for (h, lo, hi) in lst if hi - lo == DH]
                 for lst in _WINDOW_HEADS_ALL]
_STRADDLE = [(h, w, DH * h - (128 * w + 64), DH * h + DH - (128 * w + 64))
             for w in range(NW - 1) for h in range(H)
             if DH * h < 128 * (w + 1) < DH * h + DH]
_C1 = math.cos(2.0 * math.pi / 5.0)
_C2 = math.cos(4.0 * math.pi / 5.0)
_S1 = math.sin(2.0 * math.pi / 5.0)
_S2 = math.sin(4.0 * math.pi / 5.0)


def _class_freqs():
    c0 = [5 * m for m in range(65)] + [None] * 63
    c1 = [1 + 5 * m for m in range(64)] + [4 + 5 * m for m in range(64)]
    c2 = [2 + 5 * m for m in range(64)] + [3 + 5 * m for m in range(64)]
    return [c0, c1, c2]


@functools.lru_cache(maxsize=None)
def _dft_constants():
    freqs = _class_freqs()
    d2 = np.arange(128).astype(np.float64)
    norm = 1.0 / (S * D)
    fd = np.zeros((640, 256), np.float64)
    fdi = np.zeros((256, 640), np.float64)
    for lane, k in enumerate(freqs[0]):
        if k is None:
            continue
        th = 2.0 * np.pi * ((d2 * k) % D) / D
        sn = np.sin(th)
        if k == 0 or k == DF - 1:
            sn = np.zeros_like(sn)
        fd[0:128, lane] = np.cos(th)
        fd[0:128, 128 + lane] = -sn
        ck = 1.0 if (k == 0 or k == DF - 1) else 2.0
        fdi[lane, 0:128] = ck * np.cos(th) * norm
        fdi[128 + lane, 0:128] = -ck * sn * norm
    for c in (1, 2):
        rb = 128 + 256 * (c - 1)
        for lane, k in enumerate(freqs[c]):
            th = 2.0 * np.pi * ((d2 * k) % D) / D
            cs, sn = np.cos(th), np.sin(th)
            sg = 1.0 if (k % 5) == c else -1.0
            fd[rb:rb + 128, lane] = cs
            fd[rb + 128:rb + 256, lane] = sg * sn
            fd[rb:rb + 128, 128 + lane] = -sn
            fd[rb + 128:rb + 256, 128 + lane] = sg * cs
            fdi[lane, rb:rb + 128] = 2.0 * cs * norm
            fdi[128 + lane, rb:rb + 128] = -2.0 * sn * norm
            fdi[lane, rb + 128:rb + 256] = sg * 2.0 * sn * norm
            fdi[128 + lane, rb + 128:rb + 256] = sg * 2.0 * cs * norm
    g = np.zeros((N1, 3, N2, N2), np.float64)
    gi = np.zeros((N1, 3, N2, N2), np.float64)
    k2 = np.arange(N2)[:, None]
    s2 = np.arange(N2)[None, :]
    for k1 in range(N1):
        a = 2.0 * np.pi * ((s2 * (N1 * k2 + k1)) % S) / S
        c, d = np.cos(a), -np.sin(a)
        g[k1, 0], g[k1, 1], g[k1, 2] = c, d - c, c + d
        c, d = c.T, -d.T
        gi[k1, 0], gi[k1, 1], gi[k1, 2] = c, d - c, c + d
    bf = jnp.bfloat16
    return (np.asarray(fd, np.float32).astype(bf), np.asarray(fdi, np.float32).astype(bf),
            np.asarray(g, np.float32).astype(bf), np.asarray(gi, np.float32).astype(bf))


def _cmul_const(xr, xi, ang):
    c = math.cos(ang)
    s = math.sin(ang)
    eps = 1e-12
    if abs(s) < eps:
        return (xr, xi) if c > 0 else (-xr, -xi)
    if abs(c) < eps:
        return (-xi, xr) if s > 0 else (xi, -xr)
    if abs(abs(c) - abs(s)) < eps:
        r = abs(c)
        if c > 0 and s > 0:
            return (xr - xi) * r, (xr + xi) * r
        if c > 0 and s < 0:
            return (xr + xi) * r, (xi - xr) * r
        if c < 0 and s > 0:
            return (-xr - xi) * r, (xr - xi) * r
        return (xi - xr) * r, (-xr - xi) * r
    return xr * c - xi * s, xr * s + xi * c


def _dft4(x, sign):
    (ar, ai), (br, bi), (cr, ci), (dr, di) = x
    s0r, s0i = ar + cr, ai + ci
    s1r, s1i = ar - cr, ai - ci
    s2r, s2i = br + dr, bi + di
    s3r, s3i = br - dr, bi - di
    y0 = (s0r + s2r, s0i + s2i)
    y2 = (s0r - s2r, s0i - s2i)
    if sign < 0:
        tr, ti = s3i, -s3r
    else:
        tr, ti = -s3i, s3r
    y1 = (s1r + tr, s1i + ti)
    y3 = (s1r - tr, s1i - ti)
    return [y0, y1, y2, y3]


def _dft16(x, sign):
    t = []
    for b in range(4):
        col = _dft4([x[4 * a + b] for a in range(4)], sign)
        col = [_cmul_const(col[c][0], col[c][1], sign * 2.0 * math.pi * b * c / 16.0)
               for c in range(4)]
        t.append(col)
    out = [None] * 16
    for c in range(4):
        row = _dft4([t[b][c] for b in range(4)], sign)
        for d in range(4):
            out[c + 4 * d] = row[d]
    return out


def _kernel(xa_ref, wrt_ref, wit_ref, xb_ref, wqkv_hbm, wo_hbm,
            fd_hbm, fdi_hbm, g_hbm, gi_hbm,
            out_hbm,
            u0_ref, u1_ref, u2_ref, k_ref, k2_ref, vt_ref, wvt_ref, ot_ref,
            ob_ref, oa_ref, y0_ref, y1_ref, osems, asems,
            wqkv_ref, wo_ref, fd_ref, fdi_ref, g_ref, gi_ref,
            wf_ref, wtmp_ref, sems):
    t = pl.program_id(0)
    f32 = jnp.float32
    bf16 = jnp.bfloat16
    NT = (((1,), (1,)), ((), ()))
    u_refs = (u0_ref, u1_ref, u2_ref)

    copies = [
        pltpu.make_async_copy(fd_hbm, fd_ref, sems.at[0]),
        pltpu.make_async_copy(wqkv_hbm, wqkv_ref, sems.at[1]),
        pltpu.make_async_copy(wo_hbm, wo_ref, sems.at[2]),
        pltpu.make_async_copy(g_hbm, g_ref, sems.at[3]),
        pltpu.make_async_copy(gi_hbm, gi_ref, sems.at[4]),
        pltpu.make_async_copy(fdi_hbm, fdi_ref, sems.at[5]),
    ]

    @pl.when(t == 0)
    def _():
        copies[0].start()
        copies[1].start()
        ot_ref[...] = jnp.zeros((D, TQ), f32)
        copies[0].wait()

    def b_copy(step, slot):
        return pltpu.make_async_copy(
            ob_ref.at[slot],
            out_hbm.at[pl.ds(step * (RB // N2), RB // N2), :, pl.ds(D, D)],
            osems.at[slot])

    def phase1(first):
        r0 = pl.multiple_of(t * RB, RB)
        slot = t % 2
        if not first:
            @pl.when(t >= 2)
            def _():
                b_copy(t - 2, slot).wait()
        x5 = [xa_ref[:, pl.ds(128 * i, 128)].astype(f32) for i in range(5)]
        t1 = x5[1] + x5[4]
        t2 = x5[2] + x5[3]
        t3 = x5[1] - x5[4]
        t4 = x5[2] - x5[3]
        a0 = x5[0] + t1 + t2
        a1r = x5[0] + _C1 * t1 + _C2 * t2
        a1i = -(_S1 * t3 + _S2 * t4)
        a2r = x5[0] + _C2 * t1 + _C1 * t2
        a2i = -(_S2 * t3 - _S1 * t4)
        ins = [a0.astype(bf16),
               jnp.concatenate([a1r, a1i], axis=1).astype(bf16),
               jnp.concatenate([a2r, a2i], axis=1).astype(bf16)]
        for c in range(3):
            m_lo, m_n = (0, 128) if c == 0 else (128 + 256 * (c - 1), 256)
            uc = jnp.dot(ins[c], fd_ref[pl.ds(m_lo, m_n), :],
                         preferred_element_type=f32)
            u_refs[c][pl.ds(r0, RB), :] = uc
        for i, w_ref in enumerate((wrt_ref, wit_ref)):
            for b in range(RB // 128):
                wtmp_ref[b, pl.ds(0, DF), :] = (
                    w_ref[:, pl.ds(128 * b, 128)].astype(f32))
                def rows(c, n, _b=b):
                    return wtmp_ref[_b, pl.ds(c, n, stride=5), :]
                tiles = [
                    jnp.concatenate([rows(0, 65), jnp.zeros((63, 128), f32)], axis=0),
                    jnp.concatenate([rows(1, 64), rows(4, 64)], axis=0),
                    jnp.concatenate([rows(2, 64), rows(3, 64)], axis=0),
                ]
                for l in range(3):
                    wf_ref[3 * i + l, pl.ds(r0 + 128 * b, 128), :] = tiles[l].T

        if first:
            copies[1].wait()
            for c in copies[2:]:
                c.start()
            wvt_ref[...] = wqkv_ref[:, pl.ds(2 * D, D)].astype(f32).T.astype(bf16)

        xb = xb_ref[...]
        qk = jnp.dot(xb, wqkv_ref[:, pl.ds(0, 2 * D)], preferred_element_type=f32)
        q_all = (qk[:, :D] * (DH ** -0.5 * math.log2(math.e))).astype(bf16)
        k_ref[pl.ds(WIN + r0, RB), :] = qk[:, D:].astype(bf16)
        k2_ref[pl.ds(WIN + r0, RB), :] = qk[:, D + 64:2 * D - 64].astype(bf16)
        q2_all = (qk[:, 64:D - 64] * (DH ** -0.5 * math.log2(math.e))).astype(bf16)
        vt_ref[:, pl.ds(WIN + r0, RB)] = lax.dot_general(
            wvt_ref[...], xb, NT, preferred_element_type=f32).astype(bf16)

        if first:
            copies[2].wait()

        lane = lax.broadcasted_iota(jnp.int32, (1, 128), 1)
        jj = lax.broadcasted_iota(jnp.int32, (TQ, TQ), 0)
        ii = lax.broadcasted_iota(jnp.int32, (TQ, TQ), 1)
        lower = jj <= ii
        row32 = lax.broadcasted_iota(jnp.int32, (32, TQ), 0)
        NEG = -1e30

        units = [(u, j) for u in range(RB // TQ) for j in range(NW + 1)]

        def key_span(u):
            if first:
                return (2 - u) * TQ, (u + 1) * TQ
            return 0, KS

        def qk_scores(u, j):
            kofs, nk = key_span(u)
            q0 = pl.multiple_of(r0 + u * TQ + kofs, TQ)
            if j == 0:
                outs = []
                for (h, w, lo, hi) in _STRADDLE:
                    qw = q2_all[u * TQ:(u + 1) * TQ, 128 * w:128 * (w + 1)]
                    kw = k2_ref[pl.ds(q0, nk), pl.ds(128 * w, 128)]
                    qm = jnp.where((lane >= lo) & (lane < hi), qw, jnp.zeros_like(qw))
                    outs.append(lax.dot_general(kw, qm, NT,
                                                preferred_element_type=f32))
                return jnp.concatenate(outs, axis=1)
            j = j - 1
            heads = _WINDOW_HEADS[j]
            qw = q_all[u * TQ:(u + 1) * TQ, 128 * j:128 * (j + 1)]
            kw = k_ref[pl.ds(q0, nk), pl.ds(128 * j, 128)]
            qm = jnp.concatenate(
                [jnp.where((lane >= lo) & (lane < hi), qw, jnp.zeros_like(qw))
                 for (_, lo, hi) in heads], axis=0)
            return lax.dot_general(kw, qm, NT, preferred_element_type=f32)

        def finish(u, j, s_all):
            q0 = pl.multiple_of(r0 + u * TQ, TQ)
            done = _STRADDLE if j == 0 else _WINDOW_HEADS[j - 1]
            parts = [s_all[:, i * TQ:(i + 1) * TQ] for i in range(len(done))]
            for i, hd in enumerate(done):
                h = hd[0]
                s = parts[i]
                kofs, nk = key_span(u)
                if first:
                    blocks = [s[b * TQ:(b + 1) * TQ] for b in range(nk // TQ)]
                    blocks[-1] = jnp.where(lower, blocks[-1], NEG)
                    sm = blocks[0]
                    for b in blocks[1:]:
                        sm = jnp.maximum(sm, b)
                    m = jnp.max(sm, axis=0, keepdims=True)
                    pb = jnp.concatenate(
                        [jnp.exp2(b - m).astype(bf16) for b in blocks], axis=0)
                else:
                    s0, s1, s2 = s[:TQ], s[TQ:2 * TQ], s[2 * TQ:]
                    sx = jnp.where(lower, s2, s0)
                    m = jnp.max(jnp.maximum(sx, s1), axis=0, keepdims=True)
                    px = jnp.exp2(sx - m).astype(bf16)
                    p1 = jnp.exp2(s1 - m).astype(bf16)
                    zero = jnp.zeros_like(px)
                    pb = jnp.concatenate(
                        [jnp.where(lower, zero, px), p1, jnp.where(lower, px, zero)],
                        axis=0)
                a = (DH * h // 16) * 16
                off = DH * h - a
                spare = off + DH if off + DH < 32 else 0
                vt = vt_ref[pl.ds(a, 32), pl.ds(q0 + kofs, nk)]
                vt = jnp.where(lax.broadcasted_iota(jnp.int32, (32, nk), 0) == spare,
                               jnp.ones_like(vt), vt)
                oh = jnp.dot(vt, pb, preferred_element_type=f32)
                inv_l = 1.0 / oh[spare:spare + 1, :]
                rmask = (row32 >= off) & (row32 < off + DH)
                ot_ref[pl.ds(a, 32), :] = jnp.where(
                    rmask, oh * inv_l, ot_ref[pl.ds(a, 32), :])
            if j == NW:
                ot = ot_ref[...].astype(bf16)
                ob_ref[slot, u] = lax.dot_general(
                    ot, wo_ref[...], (((0,), (0,)), ((), ())),
                    preferred_element_type=f32).astype(bf16)

        s_cur = qk_scores(*units[0])
        for n, (u, j) in enumerate(units):
            s_next = qk_scores(*units[n + 1]) if n + 1 < len(units) else None
            finish(u, j, s_cur)
            s_cur = s_next
        b_copy(t, slot).start()

    @pl.when(t == 0)
    def _():
        phase1(True)

    @pl.when(t > 0)
    def _():
        phase1(False)

    @pl.when(t == NB - 1)
    def _phase2():
        for c in copies[3:]:
            c.wait()
        NP = 16

        def radix_chunk(r, l, sign=-1):
            r0 = pl.multiple_of(r * 8, 8)
            xs = []
            for b in range(N1):
                re = u_refs[l][pl.ds(b * N2 + r0, 8), pl.ds(0, 128)]
                im = u_refs[l][pl.ds(b * N2 + r0, 8), pl.ds(128, 128)]
                xs.append((re, im))
            ys = _dft16(xs, sign)
            for b in range(N1):
                u_refs[l][pl.ds(b * N2 + r0, 8), pl.ds(0, 128)] = ys[b][0]
                u_refs[l][pl.ds(b * N2 + r0, 8), pl.ds(128, 128)] = ys[b][1]

        def cmat(m_ref, k1, a, b):
            p1 = jnp.dot(m_ref[k1, 0], (a + b).astype(bf16),
                         preferred_element_type=f32)
            p2 = jnp.dot(m_ref[k1, 1], a.astype(bf16),
                         preferred_element_type=f32)
            p3 = jnp.dot(m_ref[k1, 2], b.astype(bf16),
                         preferred_element_type=f32)
            return p1 - p3, p1 + p2

        def pre(r, carry):
            radix_chunk(r, 0)
            return carry
        lax.fori_loop(0, N2 // 8, pre, 0)

        for l in range(CP // 128):
            def body(kk, carry, l=l):
                ks = [kk * NP + i for i in range(NP)]
                r0s = [pl.multiple_of(k1 * N2, N2) for k1 in ks]
                zs = [cmat(g_ref, k1, u_refs[l][pl.ds(r0, N2), pl.ds(0, 128)],
                           u_refs[l][pl.ds(r0, N2), pl.ds(128, 128)])
                      for k1, r0 in zip(ks, r0s)]
                if l + 1 < CP // 128:
                    for r in ks:
                        radix_chunk(r, l + 1)
                if l > 0:
                    for r in ks:
                        radix_chunk(r, l - 1, +1)
                vs = []
                for k1, (zr, zi) in zip(ks, zs):
                    wr = wf_ref[l, pl.ds(k1, N2, stride=N1), :]
                    wi = wf_ref[3 + l, pl.ds(k1, N2, stride=N1), :]
                    yr = zr * wr - zi * wi
                    yi = zr * wi + zi * wr
                    vs.append(cmat(gi_ref, k1, yr, yi))
                for r0, v in zip(r0s, vs):
                    u_refs[l][pl.ds(r0, N2), pl.ds(0, 128)] = v[0]
                    u_refs[l][pl.ds(r0, N2), pl.ds(128, 128)] = v[1]
                return carry
            lax.fori_loop(0, N1 // NP, body, 0)

        def inv_radix(r, y_ref):
            for sub in range(2):
                rr = pl.multiple_of(r * 16 + sub * 8, 8)
                for l in range(CP // 128 - 1, CP // 128):
                    xs = []
                    for b in range(N1):
                        re = u_refs[l][pl.ds(b * N2 + rr, 8), pl.ds(0, 128)]
                        im = u_refs[l][pl.ds(b * N2 + rr, 8), pl.ds(128, 128)]
                        xs.append((re, im))
                    ys = _dft16(xs, +1)
                    for b in range(N1):
                        y_ref[pl.ds(b * 16 + sub * 8, 8), pl.ds(256 * l, 128)] = ys[b][0]
                        y_ref[pl.ds(b * 16 + sub * 8, 8),
                              pl.ds(256 * l + 128, 128)] = ys[b][1]

        def inv_d(r, y_ref):
            cs = []
            for c in range(3):
                if c == 2:
                    yc = y_ref[:, pl.ds(256 * c, 256)].astype(bf16)
                else:
                    yc = jnp.concatenate(
                        [u_refs[c][pl.ds(b * N2 + r * 16, 16), :].astype(bf16)
                         for b in range(N1)], axis=0)
                m_lo, m_n = (0, 128) if c == 0 else (128 + 256 * (c - 1), 256)
                cs.append(jnp.dot(yc, fdi_ref[:, pl.ds(m_lo, m_n)],
                                  preferred_element_type=f32))
            c0 = cs[0]
            c1r, c1i = cs[1][:, :128], cs[1][:, 128:]
            c2r, c2i = cs[2][:, :128], cs[2][:, 128:]
            e1 = _C1 * c1r + _C2 * c2r
            f1 = _S1 * c1i + _S2 * c2i
            e2 = _C2 * c1r + _C1 * c2r
            f2 = _S2 * c1i - _S1 * c2i
            ys = [c0 + c1r + c2r, c0 + e1 - f1, c0 + e2 - f2, c0 + e2 + f2,
                  c0 + e1 + f1]
            y = jnp.concatenate(ys, axis=1).astype(bf16)
            rr = pl.multiple_of(r * 16, 16)
            oa_ref[:, pl.ds(rr, 16), :] = y.reshape(N1, 16, D)

        def a_copy(qt):
            return pltpu.make_async_copy(
                oa_ref.at[:, pl.ds(qt * 32, 32), :],
                out_hbm.at[:, pl.ds(qt * 32, 32), pl.ds(0, D)],
                asems.at[qt])

        NR = N2 // 16
        inv_radix(0, y0_ref)
        for r in range(NR):
            cur, nxt = (y0_ref, y1_ref) if r % 2 == 0 else (y1_ref, y0_ref)
            if r + 1 < NR:
                inv_radix(r + 1, nxt)
            inv_d(r, cur)
            if r % 2 == 1:
                a_copy(r // 2).start()
        b_copy(NB - 2, (NB - 2) % 2).wait()
        b_copy(NB - 1, (NB - 1) % 2).wait()
        for qt in range(NR // 2):
            a_copy(qt).wait()


@jax.jit
def pallas_concat_heads__spectral_gfnet__sliding_block__prompt_kernel(
    A_x: jax.Array,
    A_w_r: jax.Array,
    A_w_i: jax.Array,
    B_x: jax.Array,
    B_wqkv: jax.Array,
    B_wo: jax.Array,
):
    bf16 = jnp.bfloat16
    fd, fdi, g, gi = _dft_constants()
    xa = A_x.reshape(S, D)
    xb = B_x.reshape(S, D)

    row_spec = pl.BlockSpec((RB, D), lambda t: (t, 0))
    any_spec = pl.BlockSpec(memory_space=pl.ANY)
    wt_spec = pl.BlockSpec((DF, RB), lambda t: (0, t))

    out = pl.pallas_call(
        _kernel,
        grid=(NB,),
        in_specs=[row_spec, wt_spec, wt_spec, row_spec, any_spec, any_spec,
                  any_spec, any_spec, any_spec, any_spec],
        out_specs=any_spec,
        out_shape=jax.ShapeDtypeStruct((N1, N2, 2 * D), bf16),
        scratch_shapes=[
            pltpu.VMEM((S, 256), jnp.float32),
            pltpu.VMEM((S, 256), jnp.float32),
            pltpu.VMEM((S, 256), jnp.float32),
            pltpu.VMEM((S + WIN, D), bf16),
            pltpu.VMEM((S + WIN, D - 128), bf16),
            pltpu.VMEM((D, S + WIN), bf16),
            pltpu.VMEM((D, D), bf16),
            pltpu.VMEM((D, TQ), jnp.float32),
            pltpu.VMEM((2, RB // N2, N2, D), bf16),
            pltpu.VMEM((N1, N2, D), bf16),
            pltpu.VMEM((256, 2 * CP), jnp.float32),
            pltpu.VMEM((256, 2 * CP), jnp.float32),
            pltpu.SemaphoreType.DMA((2,)),
            pltpu.SemaphoreType.DMA((4,)),
            pltpu.VMEM((D, 3 * D), bf16),
            pltpu.VMEM((D, D), bf16),
            pltpu.VMEM((D, 256), bf16),
            pltpu.VMEM((256, D), bf16),
            pltpu.VMEM((N1, 3, N2, N2), bf16),
            pltpu.VMEM((N1, 3, N2, N2), bf16),
            pltpu.VMEM((6, S, 128), jnp.float32),
            pltpu.VMEM((RB // 128, 328, 128), jnp.float32),
            pltpu.SemaphoreType.DMA((6,)),
        ],
        compiler_params=pltpu.CompilerParams(
            dimension_semantics=("arbitrary",),
            vmem_limit_bytes=126 * 1024 * 1024,
        ),
    )(xa, A_w_r.T, A_w_i.T, xb, B_wqkv, B_wo, fd, fdi, g, gi)
    return out.reshape(1, S, 2 * D)
```
